```python
import os as _os
_os.environ.setdefault("JAX_PLATFORMS", "cpu")
import jax
import jax.numpy as jnp

def _softmax(x, axis=-1):
    return jax.nn.softmax(x, axis=axis)
def _gelu(x):
    return jax.nn.gelu(x, approximate=True)
def _silu(x):
    return jax.nn.silu(x)
def _sigmoid(x):
    return jax.nn.sigmoid(x)
def _layernorm(x, axis=-1, eps=1e-5):
    m = jnp.mean(x, axis=axis, keepdims=True)
    v = jnp.var(x, axis=axis, keepdims=True)
    return (x - m) / jnp.sqrt(v + eps)
def _scatter_add(tgt, idx, src, axis=0):
    return tgt.at[idx].add(src)
def _segment_sum(src, seg, n):
    return jax.ops.segment_sum(src, seg, n)
class _Rng:
    def __init__(self, key):
        self._k = key
    def _next(self):
        self._k, sub = jax.random.split(self._k)
        return sub
    def normal(self, shape):
        return jax.random.normal(self._next(), shape, dtype=jnp.bfloat16)
    def randint(self, lo, hi, shape):
        return jax.random.randint(self._next(), shape, lo, hi, dtype=jnp.int32)
    def uniform(self, shape, lo=0.0, hi=1.0):
        return jax.random.uniform(self._next(), shape, jnp.bfloat16, lo, hi)
    def permutation(self, n):
        return jax.random.permutation(self._next(), n)


kernel_name = 'standalone__channel_attn_cbam__vision'

def setup_inputs():
    _rng = _Rng(jax.random.key(int.from_bytes(__import__("os").urandom(4), "little")))
    _w = (lambda a: (lambda t: t.astype(jnp.bfloat16) if jnp.issubdtype(t.dtype, jnp.floating) else t)(jnp.asarray(a)))
    H = W = 384
    C = 192
    r = max(C // 4, 1)
    return {
        "x": _w((lambda *s: _rng.normal(s) * 0.2)(1, H, W, C) + (lambda *s: _rng.normal(s) * 0.2)(1, 1, 1, C) * 2.0),
        "w1": _w((lambda *s: _rng.normal(s) * 0.2)(C, r)),
        "w2": _w((lambda *s: _rng.normal(s) * 0.2)(r, C)),
    }

def reference(x, w1, w2):
    B, H, W, C = x.shape
    xf = x.reshape(B, H * W, C)
    gap = jnp.mean(xf, 1)
    gmp = jnp.amax(xf, 1)
    h_a = gap @ w1
    h_a = h_a * (lambda x, dt: x.astype(dt))(h_a > 0, h_a.dtype)
    h_m = gmp @ w1
    h_m = h_m * (lambda x, dt: x.astype(dt))(h_m > 0, h_m.dtype)
    scale = _sigmoid(h_a @ w2 + h_m @ w2)
    return x * scale[:, None, None, :]
```

```python
import functools

import jax
import jax.numpy as jnp
from jax import lax
import jax.experimental.pallas as pl
import jax.experimental.pallas.tpu as pltpu

_LANES = 128
_J = 12
_QC = 48
_CG = 96


def _kernel(x_hbm, w1t_hbm, w2_hbm, o_hbm,
            xbuf, w1buf, w2buf, sum_ref, max_ref, scale_ref,
            in_sems, w_sems, out_sem, *, read_chunks, first_splits):
    A, J, C, W = xbuf.shape
    n_lane_tiles = W // _LANES
    f32 = jnp.float32
    bf16 = jnp.bfloat16

    def read_copy(i):
        a0, na, j0, nj = read_chunks[i]
        sl = (pl.ds(a0, na), pl.ds(j0, nj))
        return pltpu.make_async_copy(x_hbm.at[sl], xbuf.at[sl], in_sems.at[i])

    w1_copy = pltpu.make_async_copy(w1t_hbm, w1buf, w_sems.at[0])
    w2_copy = pltpu.make_async_copy(w2_hbm, w2buf, w_sems.at[1])
    read_copy(0).start()
    w1_copy.start()
    w2_copy.start()
    for i in range(1, len(read_chunks)):
        read_copy(i).start()

    sum_ref[...] = jnp.zeros(sum_ref.shape, f32)
    max_ref[...] = jnp.full(max_ref.shape, -jnp.inf, f32)

    def reduce_chunk(a0, na, j0, nj):
        n = na * nj
        for g in range(C // _CG):
            cs = pl.ds(g * _CG, _CG)

            def body(t, carry):
                s, m = carry
                if na == 1:
                    a, j = a0, j0 + t
                else:
                    a, j = a0 + t // nj, j0 + t % nj
                v = xbuf[a, j, cs, :].astype(f32)
                parts = [v[:, k * _LANES:(k + 1) * _LANES]
                         for k in range(n_lane_tiles)]
                ps, pm = parts[0], parts[0]
                for p in parts[1:]:
                    ps = ps + p
                    pm = jnp.maximum(pm, p)
                return s + ps, jnp.maximum(m, pm)

            s, m = lax.fori_loop(0, n, body, (sum_ref[cs, :], max_ref[cs, :]),
                                 unroll=2)
            sum_ref[cs, :] = s
            max_ref[cs, :] = m

    for i, ch in enumerate(read_chunks):
        read_copy(i).wait()
        reduce_chunk(*ch)

    w1_copy.wait()
    w2_copy.wait()
    inv_n = 1.0 / (A * J * W)
    gap = jnp.sum(sum_ref[...], axis=1, keepdims=True) * inv_n
    gmp = jnp.max(max_ref[...], axis=1, keepdims=True)
    g = jnp.concatenate(
        [jnp.broadcast_to(gap, (C, _LANES)), jnp.broadcast_to(gmp, (C, _LANES))],
        axis=1).astype(bf16)
    h = jnp.dot(w1buf[...], g, preferred_element_type=f32).astype(bf16)
    h = jnp.maximum(h.astype(f32), 0.0).astype(bf16)
    s = lax.dot_general(w2buf[...], h, (((0,), (0,)), ((), ())),
                        preferred_element_type=f32)
    s = s.astype(bf16).astype(f32)
    z = (s[:, :_LANES] + s[:, _LANES:]).astype(bf16).astype(f32)
    scale_ref[...] = jax.nn.sigmoid(z).astype(bf16).astype(f32)

    def scale_and_write(j, q, a0, na):
        c0 = q * _QC
        if not isinstance(c0, int):
            c0 = pl.multiple_of(c0, 16)
        cs = pl.ds(c0, _QC)
        sc = scale_ref[cs, :]
        sc = jnp.concatenate([sc] * n_lane_tiles, axis=1)

        def body(t, _):
            a = a0 + t
            xbuf[a, j, cs, :] = (xbuf[a, j, cs, :].astype(f32) * sc).astype(bf16)
            return 0

        lax.fori_loop(0, na, body, 0, unroll=min(na, 4))
        sl = (pl.ds(a0, na), j, cs)
        pltpu.make_async_copy(xbuf.at[sl], o_hbm.at[sl], out_sem).start()

    nq = C // _QC
    for a0, na in first_splits:
        scale_and_write(0, 0, a0, na)

    def chunk_body(k, _):
        scale_and_write(k // nq, k % nq, 0, A)
        return 0

    lax.fori_loop(1, J * nq, chunk_body, 0)
    pltpu.make_async_copy(xbuf, o_hbm, out_sem).wait()


@jax.jit
def pallas_standalone__channel_attn_cbam__vision_kernel(
    x: jax.Array,
    w1: jax.Array,
    w2: jax.Array,
):
    B, H, W, C = x.shape
    r = w1.shape[1]
    assert B == 1 and H % _J == 0 and W % _LANES == 0
    assert C % _QC == 0 and C % _CG == 0
    A = H // _J
    xt = jnp.transpose(x, (0, 1, 3, 2)).reshape(A, _J, C, W)
    w1t = jnp.transpose(w1)

    read_chunks = ((0, 8, 0, _J), (8, 8, 0, _J), (16, 8, 0, _J), (24, 6, 0, _J),
                   (30, 1, 0, _J), (31, 1, 0, 8), (31, 1, 8, 2), (31, 1, 10, 2))
    first_splits = ((0, 2), (2, 6), (8, 24))

    out = pl.pallas_call(
        functools.partial(_kernel, read_chunks=read_chunks,
                          first_splits=first_splits),
        out_shape=jax.ShapeDtypeStruct((A, _J, C, W), x.dtype),
        in_specs=[pl.BlockSpec(memory_space=pl.ANY)] * 3,
        out_specs=pl.BlockSpec(memory_space=pl.ANY),
        scratch_shapes=[
            pltpu.VMEM((A, _J, C, W), x.dtype),
            pltpu.VMEM((r, C), w1.dtype),
            pltpu.VMEM((r, C), w2.dtype),
            pltpu.VMEM((C, _LANES), jnp.float32),
            pltpu.VMEM((C, _LANES), jnp.float32),
            pltpu.VMEM((C, _LANES), jnp.float32),
            pltpu.SemaphoreType.DMA((len(read_chunks),)),
            pltpu.SemaphoreType.DMA((2,)),
            pltpu.SemaphoreType.DMA(()),
        ],
        compiler_params=pltpu.CompilerParams(
            vmem_limit_bytes=100 * 1024 * 1024),
    )(xt, w1t, w2)
    return jnp.transpose(out.reshape(B, H, C, W), (0, 1, 3, 2))
```

```python
import functools

import jax
import jax.numpy as jnp
from jax import lax
import jax.experimental.pallas as pl
import jax.experimental.pallas.tpu as pltpu

_LANES = 128
_TR = 8
_S = 256
_BLK = 8


def _kernel(x_hbm, w1t_hbm, w2_hbm, o_hbm,
            xbuf, w1buf, w2buf, w1d_ref, w2d_ref, sum_ref, max_ref, tab_ref,
            flag_ref, out_sem, *, cfg):
    A = xbuf.shape[0]
    ng = sum_ref.shape[0]
    C = ng * _TR
    nw = cfg["nw"]
    P = ng * nw
    nb = P // _BLK
    bpa = _S // _BLK
    brows = _BLK * _TR
    vrows = _S * _TR
    hrows = P * _TR
    grows = nw * _TR
    H = A * _S // P
    half = _LANES // 2
    f32 = jnp.float32
    bf16 = jnp.bfloat16
    bulk = cfg["bulk"]
    K, nl = cfg["K"], cfg["nl"]
    ne = ng - nl
    U = cfg["p1_unroll"]

    def pieces(r0, r1):
        out = []
        while r0 < r1:
            a, r = divmod(r0, vrows)
            n = min(r1 - r0, vrows - r)
            out.append((a, r, n))
            r0 += n
        return out

    def phase1(in_sems, w_sems):
        nbulk = len(bulk) - 1
        tail0 = bulk[-1] * vrows

        def bulk_copy(i):
            sl = pl.ds(bulk[i], bulk[i + 1] - bulk[i])
            return pltpu.make_async_copy(x_hbm.at[sl], xbuf.at[sl], in_sems.at[i])

        def tail_copies(ranges, sem):
            cs = []
            for r0, r1 in ranges:
                for a, r, n in pieces(max(r0, tail0), r1):
                    sl = (a, pl.ds(r, n))
                    cs.append(pltpu.make_async_copy(
                        x_hbm.at[sl], xbuf.at[sl], sem))
            return cs

        early = [(h * hrows, h * hrows + ne * grows) for h in range(H - K, H)]
        late = [(h * hrows + ne * grows, (h + 1) * hrows)
                for h in range(H - K, H)]
        assert (H - K) * hrows <= tail0 <= late[0][0]
        e1_cs = tail_copies(early[:-1], in_sems.at[nbulk])
        e2_cs = tail_copies(early[-1:], in_sems.at[nbulk + 1])
        l1_cs = tail_copies(late[:-1], in_sems.at[nbulk + 2])
        l2_cs = tail_copies(late[-1:], in_sems.at[nbulk + 3])

        w1_copy = pltpu.make_async_copy(w1t_hbm, w1buf, w_sems.at[0])
        w2_copy = pltpu.make_async_copy(w2_hbm, w2buf, w_sems.at[1])
        bulk_copy(0).start()
        bulk_copy(1).start()
        w1_copy.start()
        w2_copy.start()

        flag_ref[0] = 1

        def prep_weights():
            r = w1buf.shape[0]
            w1_copy.wait()
            w2_copy.wait()
            row = lax.broadcasted_iota(jnp.int32, (r, _LANES), 0)
            col = lax.broadcasted_iota(jnp.int32, (r, _LANES), 1)
            dup = jnp.where((col == row) | (col == row + half), 1.0, 0.0)
            dup = dup.astype(bf16)
            tn = (((0,), (0,)), ((), ()))
            w1d_ref[...] = lax.dot_general(w1buf[...], dup, tn,
                                           preferred_element_type=f32)
            w2d_ref[...] = lax.dot_general(w2buf[...], dup, tn,
                                           preferred_element_type=f32)

        def accumulate(v, s, m):
            v = v.reshape(s.shape[0], nw, _TR, _LANES)
            ps, pm = v[:, 0], v[:, 0]
            for k in range(1, nw):
                ps = ps + v[:, k]
                pm = jnp.maximum(pm, v[:, k])
            return s + ps, jnp.maximum(m, pm)

        def load_block(beta):
            a = lax.shift_right_logical(beta, bpa.bit_length() - 1)
            r = pl.multiple_of(lax.bitwise_and(beta, bpa - 1) * brows, brows)
            return xbuf[a, pl.ds(r, brows), :].astype(f32)

        def reduce_rows(h0, h1):
            for g in range(nb // nw):
                gs = pl.ds(g * _BLK, _BLK)

                def body(t, c):
                    for k in range(U):
                        b0 = (h0 + t * U + k) * nb + g * nw
                        v = jnp.concatenate(
                            [load_block(b0 + i) for i in range(nw)], axis=0)
                        c = accumulate(v, *c)
                    return c

                if h0 == 0:
                    acc = (_BLK, _TR, _LANES)
                    init = (jnp.zeros(acc, f32), jnp.full(acc, -jnp.inf, f32))
                else:
                    init = (sum_ref[gs], max_ref[gs])
                s, m = lax.fori_loop(0, (h1 - h0) // U, body, init)
                sum_ref[gs] = s
                max_ref[gs] = m

        def fold_static(hs, g0, g1, s, m):
            for h in hs:
                v = jnp.concatenate(
                    [xbuf[a, pl.ds(r, n), :].astype(f32) for a, r, n in
                     pieces(h * hrows + g0 * grows, h * hrows + g1 * grows)],
                    axis=0)
                s, m = accumulate(v, s, m)
            return s, m

        done = 0
        for i in range(nbulk):
            bulk_copy(i).wait()
            if i == 0:
                for k in range(2, nbulk):
                    bulk_copy(k).start()
                for c in e1_cs + e2_cs + l1_cs + l2_cs:
                    c.start()
            if i == 1:
                prep_weights()
            h1 = min(bulk[i + 1] * vrows // hrows, H - K)
            h1 -= (h1 - done) % U
            reduce_rows(done, h1)
            done = h1
        assert done == H - K

        inv_n = 1.0 / (H * nw * _LANES)

        def hidden_part(g0, s, m):
            n = s.shape[0]
            s = s.reshape(n * _TR, _LANES)
            m = m.reshape(n * _TR, _LANES)
            gap = jnp.sum(s, axis=1, keepdims=True) * inv_n
            gmp = jnp.max(m, axis=1, keepdims=True)
            lane = lax.broadcasted_iota(jnp.int32, s.shape, 1)
            g = jnp.where(lane < half, gap, gmp).astype(bf16).astype(f32)
            hp = g * w1d_ref[pl.ds(g0 * _TR, n * _TR), :]
            parts = [hp[k * _TR:(k + 1) * _TR] for k in range(n)]
            while len(parts) > 1:
                parts = [parts[k] + parts[k + 1] if k + 1 < len(parts)
                         else parts[k] for k in range(0, len(parts), 2)]
            return parts[0]

        sub = cfg["sub"]
        subs = [(g0, min(g0 + sub, ne)) for g0 in range(0, ne, sub)]
        for c in e1_cs:
            c.wait()
        for g0, g1 in subs:
            gs = pl.ds(g0, g1 - g0)
            s, m = fold_static(range(H - K, H - 1), g0, g1,
                               sum_ref[gs], max_ref[gs])
            sum_ref[gs] = s
            max_ref[gs] = m
        for c in e2_cs:
            c.wait()
        hacc = None
        for g0, g1 in subs:
            gs = pl.ds(g0, g1 - g0)
            s, m = fold_static([H - 1], g0, g1, sum_ref[gs], max_ref[gs])
            p = hidden_part(g0, s, m)
            hacc = p if hacc is None else hacc + p
        for c in l1_cs:
            c.wait()
        gs = pl.ds(ne, nl)
        s, m = fold_static(range(H - K, H - 1), ne, ng, sum_ref[gs], max_ref[gs])
        for c in l2_cs:
            c.wait()
        s, m = fold_static([H - 1], ne, ng, s, m)
        hacc = hacc + hidden_part(ne, s, m)
        h = jnp.sum(hacc, axis=0, keepdims=True)
        h = jnp.maximum(h.astype(bf16).astype(f32), 0.0)

        G = cfg["G"]
        o = cfg["o"]
        es = o + 17
        order = list(range(1, es // nw + 1)) + [0] + list(range(es // nw + 1, ng))
        sc_g = {}
        for k in order:
            z = jnp.sum(w2d_ref[pl.ds(k * _TR, _TR), :] * h, axis=1,
                        keepdims=True)
            z = jnp.broadcast_to(z, (_TR, _LANES)).astype(bf16).astype(f32)
            sc_g[k] = (0.5 * jnp.tanh(0.5 * z) + 0.5).astype(bf16).astype(f32)

        def write(a0, na, b0, n):
            sl = (pl.ds(a0, na), pl.ds(b0 * _TR, n * _TR))
            pltpu.make_async_copy(xbuf.at[sl], o_hbm.at[sl], out_sem).start()

        def scale_static(a, e0, n):
            sc = jnp.concatenate(
                [sc_g[((a * _S + t) // nw) % ng] for t in range(e0, e0 + n)],
                axis=0)
            rs = pl.ds(e0 * _TR, n * _TR)
            xbuf[a, rs, :] = (xbuf[a, rs, :].astype(f32) * sc).astype(bf16)

        def head_static(a0, n):
            for a in range(a0, a0 + n):
                scale_static(a, 0, es)
            write(a0, n, o, 17)
            write(a0, n, 0, o)

        ramp = cfg["ramp"]
        head_static(0, ramp[0])

        @pl.when(flag_ref[0] == 1)
        def _():
            a0 = ramp[0]
            for n in ramp[1:]:
                head_static(a0, n)
                a0 += n
            assert a0 == G

        @pl.when(flag_ref[0] == 1)
        def _():
            for t in range(tab_ref.shape[0] // _TR):
                tab_ref[pl.ds(t * _TR, _TR), :] = sc_g[(t // nw) % ng]

        step = _S % P

        def wrap(p):
            return jnp.where(p >= P, p - P, p)

        def scale_block(a0, pos0, e0, n):
            p = lax.rem(pos0 + e0, P)
            r0 = e0 * _TR
            if not isinstance(r0, int):
                r0 = pl.multiple_of(r0, 2 * _TR)
            rs = pl.ds(r0, n * _TR)
            for j in range(G):
                sc = tab_ref[pl.ds(pl.multiple_of(p * _TR, _TR), n * _TR), :]
                xbuf[a0 + j, rs, :] = (
                    xbuf[a0 + j, rs, :].astype(f32) * sc).astype(bf16)
                p = wrap(p + step)

        nper = (_S - es) // 32
        last = es + 32 * nper

        def group(g, pos0):
            a0 = g * G

            @pl.when(g > 0)
            def _():
                scale_block(a0, pos0, 0, es)
                write(a0, G, 0, o)
                write(a0, G, o, 17)

            def period(mi, _):
                e0 = es + 32 * mi
                scale_block(a0, pos0, e0, 16)
                write(a0, G, e0, 15)
                scale_block(a0, pos0, e0 + 16, 16)
                write(a0, G, e0 + 15, 17)
                return 0

            lax.fori_loop(0, nper, period, 0)
            scale_block(a0, pos0, last, _S - last)
            write(a0, G, last, _S - last)
            return lax.rem(pos0 + G * step, P)

        lax.fori_loop(0, A // G, group, jnp.int32(0))

    pl.run_scoped(phase1,
                  pltpu.SemaphoreType.DMA((len(bulk) + 3,)),
                  pltpu.SemaphoreType.DMA((2,)))
    pltpu.make_async_copy(xbuf, o_hbm, out_sem).wait()


def build(o=5, G=6, ramp=(1, 2, 3), p1_unroll=4, K=4, nl=6, sub=6,
          bulk=(0, 20, 72, 98, 105, 107), name=None):
    assert o % 2 == 1 and o + 17 < 32

    def fn(x, w1, w2):
        B, H, W, C = x.shape
        r = w1.shape[1]
        nw = W // _LANES
        ng = C // _TR
        A = H * ng * nw // _S
        xt = jnp.transpose(x, (0, 1, 3, 2))
        xf = xt.reshape(H * ng, _TR, nw, _LANES).transpose(0, 2, 1, 3)
        xf = xf.reshape(A, _S * _TR, _LANES)
        w1t = jnp.transpose(w1)
        cfg = dict(nw=nw, bulk=bulk, p1_unroll=p1_unroll, K=K, nl=nl, sub=sub,
                   G=G, o=o, ramp=ramp)
        out = pl.pallas_call(
            functools.partial(_kernel, cfg=cfg),
            out_shape=jax.ShapeDtypeStruct(xf.shape, x.dtype),
            in_specs=[pl.BlockSpec(memory_space=pl.ANY)] * 3,
            out_specs=pl.BlockSpec(memory_space=pl.ANY),
            scratch_shapes=[
                pltpu.VMEM(xf.shape, x.dtype),
                pltpu.VMEM((r, C), w1.dtype),
                pltpu.VMEM((r, C), w2.dtype),
                pltpu.VMEM((C, _LANES), jnp.float32),
                pltpu.VMEM((C, _LANES), jnp.float32),
                pltpu.VMEM((ng, _TR, _LANES), jnp.float32),
                pltpu.VMEM((ng, _TR, _LANES), jnp.float32),
                pltpu.VMEM(((ng * nw + o + 17) * _TR, _LANES), jnp.float32),
                pltpu.SMEM((1,), jnp.int32),
                pltpu.SemaphoreType.DMA(()),
            ],
            compiler_params=pltpu.CompilerParams(
                vmem_limit_bytes=100 * 1024 * 1024),
            name=name,
        )(xf, w1t, w2)
        out = out.reshape(H * ng, nw, _TR, _LANES).transpose(0, 2, 1, 3)
        return jnp.transpose(out.reshape(B, H, C, W), (0, 1, 3, 2))
    return fn


pallas_standalone__channel_attn_cbam__vision_kernel = jax.jit(build(p1_unroll=2, bulk=(0,20,64,90,101,105,106,107)))
```

```python
import functools

import jax
import jax.numpy as jnp
from jax import lax
import jax.experimental.pallas as pl
import jax.experimental.pallas.tpu as pltpu

_LANES = 128
_TR = 8
_S = 256
_BLK = 8
_U = 2
_BULK = (0, 20, 64, 90, 101, 105, 106, 107)
_K = 4
_NL = 6
_SUB = 6
_G = 6
_PER = 32
_O = 5
_L1 = 13
_RAMP = (1, 2, 3)


def _kernel(x_hbm, w1t_hbm, w2_hbm, o_hbm,
            xbuf, w1buf, w2buf, w1d_ref, w2d_ref, sum_ref, max_ref, tab_ref,
            flag_ref, *, nw):
    A = xbuf.shape[0]
    ng = sum_ref.shape[0]
    P = ng * nw
    nb = P // _BLK
    bpa = _S // _BLK
    brows = _BLK * _TR
    vrows = _S * _TR
    hrows = P * _TR
    grows = nw * _TR
    H = A * _S // P
    half = _LANES // 2
    ne = ng - _NL
    nbulk = len(_BULK) - 1
    f32 = jnp.float32
    bf16 = jnp.bfloat16

    def pieces(r0, r1):
        out = []
        while r0 < r1:
            a, r = divmod(r0, vrows)
            n = min(r1 - r0, vrows - r)
            out.append((a, r, n))
            r0 += n
        return out

    def body(in_sems, w_sems, out_sem):
        tail0 = _BULK[-1] * vrows

        def bulk_copy(i):
            sl = pl.ds(_BULK[i], _BULK[i + 1] - _BULK[i])
            return pltpu.make_async_copy(x_hbm.at[sl], xbuf.at[sl],
                                         in_sems.at[i])

        def tail_copies(ranges, sem):
            cs = []
            for r0, r1 in ranges:
                for a, r, n in pieces(max(r0, tail0), r1):
                    sl = (a, pl.ds(r, n))
                    cs.append(pltpu.make_async_copy(x_hbm.at[sl], xbuf.at[sl],
                                                    sem))
            return cs

        early = [(h * hrows, h * hrows + ne * grows) for h in range(H - _K, H)]
        late = [(h * hrows + ne * grows, (h + 1) * hrows)
                for h in range(H - _K, H)]
        assert (H - _K) * hrows <= tail0 <= late[0][0]
        e1_cs = tail_copies(early[:-1], in_sems.at[nbulk])
        e2_cs = tail_copies(early[-1:], in_sems.at[nbulk + 1])
        l1_cs = tail_copies(late[:-1], in_sems.at[nbulk + 2])
        l2_cs = tail_copies(late[-1:], in_sems.at[nbulk + 3])

        w1_copy = pltpu.make_async_copy(w1t_hbm, w1buf, w_sems.at[0])
        w2_copy = pltpu.make_async_copy(w2_hbm, w2buf, w_sems.at[1])
        bulk_copy(0).start()
        bulk_copy(1).start()
        w1_copy.start()
        w2_copy.start()

        flag_ref[0] = 1

        def prep_weights():
            r = w1buf.shape[0]
            w1_copy.wait()
            w2_copy.wait()
            row = lax.broadcasted_iota(jnp.int32, (r, _LANES), 0)
            col = lax.broadcasted_iota(jnp.int32, (r, _LANES), 1)
            dup = jnp.where((col == row) | (col == row + half), 1.0, 0.0)
            dup = dup.astype(bf16)
            tn = (((0,), (0,)), ((), ()))
            w1d_ref[...] = lax.dot_general(w1buf[...], dup, tn,
                                           preferred_element_type=f32)
            w2d_ref[...] = lax.dot_general(w2buf[...], dup, tn,
                                           preferred_element_type=f32)

        def accumulate(v, s, m):
            v = v.reshape(s.shape[0], nw, _TR, _LANES)
            ps, pm = v[:, 0], v[:, 0]
            for k in range(1, nw):
                ps = ps + v[:, k]
                pm = jnp.maximum(pm, v[:, k])
            return s + ps, jnp.maximum(m, pm)

        def load_block(beta):
            a = lax.shift_right_logical(beta, bpa.bit_length() - 1)
            r = pl.multiple_of(lax.bitwise_and(beta, bpa - 1) * brows, brows)
            return xbuf[a, pl.ds(r, brows), :].astype(f32)

        def reduce_rows(h0, h1):
            for g in range(nb // nw):
                gs = pl.ds(g * _BLK, _BLK)

                def step(t, c):
                    for k in range(_U):
                        b0 = (h0 + t * _U + k) * nb + g * nw
                        v = jnp.concatenate(
                            [load_block(b0 + i) for i in range(nw)], axis=0)
                        c = accumulate(v, *c)
                    return c

                if h0 == 0:
                    acc = (_BLK, _TR, _LANES)
                    init = (jnp.zeros(acc, f32), jnp.full(acc, -jnp.inf, f32))
                else:
                    init = (sum_ref[gs], max_ref[gs])
                s, m = lax.fori_loop(0, (h1 - h0) // _U, step, init)
                sum_ref[gs] = s
                max_ref[gs] = m

        def fold_static(hs, g0, g1, s, m):
            for h in hs:
                v = jnp.concatenate(
                    [xbuf[a, pl.ds(r, n), :].astype(f32) for a, r, n in
                     pieces(h * hrows + g0 * grows, h * hrows + g1 * grows)],
                    axis=0)
                s, m = accumulate(v, s, m)
            return s, m

        done = 0
        for i in range(nbulk):
            bulk_copy(i).wait()
            if i == 0:
                for k in range(2, nbulk):
                    bulk_copy(k).start()
                for c in e1_cs + e2_cs + l1_cs + l2_cs:
                    c.start()
            if i == 1:
                prep_weights()
            h1 = min(_BULK[i + 1] * vrows // hrows, H - _K)
            h1 -= (h1 - done) % _U
            reduce_rows(done, h1)
            done = h1
        assert done == H - _K

        inv_n = 1.0 / (H * nw * _LANES)

        def hidden_part(g0, s, m):
            n = s.shape[0]
            s = s.reshape(n * _TR, _LANES)
            m = m.reshape(n * _TR, _LANES)
            gap = jnp.sum(s, axis=1, keepdims=True) * inv_n
            gmp = jnp.max(m, axis=1, keepdims=True)
            lane = lax.broadcasted_iota(jnp.int32, s.shape, 1)
            g = jnp.where(lane < half, gap, gmp).astype(bf16).astype(f32)
            hp = g * w1d_ref[pl.ds(g0 * _TR, n * _TR), :]
            parts = [hp[k * _TR:(k + 1) * _TR] for k in range(n)]
            while len(parts) > 1:
                parts = [parts[k] + parts[k + 1] if k + 1 < len(parts)
                         else parts[k] for k in range(0, len(parts), 2)]
            return parts[0]

        subs = [(g0, min(g0 + _SUB, ne)) for g0 in range(0, ne, _SUB)]
        for c in e1_cs:
            c.wait()
        for g0, g1 in subs:
            gs = pl.ds(g0, g1 - g0)
            s, m = fold_static(range(H - _K, H - 1), g0, g1,
                               sum_ref[gs], max_ref[gs])
            sum_ref[gs] = s
            max_ref[gs] = m
        for c in e2_cs:
            c.wait()
        hacc = None
        for g0, g1 in subs:
            gs = pl.ds(g0, g1 - g0)
            s, m = fold_static([H - 1], g0, g1, sum_ref[gs], max_ref[gs])
            p = hidden_part(g0, s, m)
            hacc = p if hacc is None else hacc + p
        for c in l1_cs:
            c.wait()
        gs = pl.ds(ne, _NL)
        s, m = fold_static(range(H - _K, H - 1), ne, ng,
                           sum_ref[gs], max_ref[gs])
        for c in l2_cs:
            c.wait()
        s, m = fold_static([H - 1], ne, ng, s, m)
        hacc = hacc + hidden_part(ne, s, m)
        h = jnp.sum(hacc, axis=0, keepdims=True)
        h = jnp.maximum(h.astype(bf16).astype(f32), 0.0)

        l2 = _PER - _L1
        es = _O + _L1
        order = (list(range(1, es // nw + 1)) + [0]
                 + list(range(es // nw + 1, ng)))
        sc_g = {}
        for k in order:
            z = jnp.sum(w2d_ref[pl.ds(k * _TR, _TR), :] * h, axis=1,
                        keepdims=True)
            z = jnp.broadcast_to(z, (_TR, _LANES)).astype(bf16).astype(f32)
            sc_g[k] = (0.5 * jnp.tanh(0.5 * z) + 0.5).astype(bf16).astype(f32)

        def write(a0, na, b0, n):
            sl = (pl.ds(a0, na), pl.ds(b0 * _TR, n * _TR))
            pltpu.make_async_copy(xbuf.at[sl], o_hbm.at[sl], out_sem).start()

        def head_static(a0, n):
            rs = pl.ds(0, es * _TR)
            for a in range(a0, a0 + n):
                sc = jnp.concatenate(
                    [sc_g[((a * _S + t) // nw) % ng] for t in range(es)],
                    axis=0)
                xbuf[a, rs, :] = (xbuf[a, rs, :].astype(f32) * sc).astype(bf16)
            write(a0, n, _O, _L1)
            write(a0, n, 0, _O)

        head_static(0, _RAMP[0])

        @pl.when(flag_ref[0] == 1)
        def _():
            a0 = _RAMP[0]
            for n in _RAMP[1:]:
                head_static(a0, n)
                a0 += n
            assert a0 == _G

        @pl.when(flag_ref[0] == 1)
        def _():
            for t in range(tab_ref.shape[0] // _TR):
                tab_ref[pl.ds(t * _TR, _TR), :] = sc_g[(t // nw) % ng]

        adv = _S % P

        def scale_block(a0, pos0, e0, n):
            p = lax.rem(pos0 + e0, P)
            r0 = e0 * _TR
            if not isinstance(r0, int):
                r0 = pl.multiple_of(r0, 2 * _TR)
            rs = pl.ds(r0, n * _TR)
            for j in range(_G):
                sc = tab_ref[pl.ds(pl.multiple_of(p * _TR, _TR), n * _TR), :]
                xbuf[a0 + j, rs, :] = (
                    xbuf[a0 + j, rs, :].astype(f32) * sc).astype(bf16)
                p = p + adv
                p = jnp.where(p >= P, p - P, p)

        nper = (_S - es) // _PER
        last = es + _PER * nper

        def group(g, pos0):
            a0 = g * _G

            @pl.when(g > 0)
            def _():
                scale_block(a0, pos0, 0, es)
                write(a0, _G, 0, _O)
                write(a0, _G, _O, _L1)

            def period(mi, _):
                e0 = es + _PER * mi
                scale_block(a0, pos0, e0, l2 + 1)
                write(a0, _G, e0, l2)
                scale_block(a0, pos0, e0 + l2 + 1, _L1 - 1)
                write(a0, _G, e0 + l2, _L1)
                return 0

            lax.fori_loop(0, nper, period, 0)
            scale_block(a0, pos0, last, _S - last)
            write(a0, _G, last, _S - last)
            return lax.rem(pos0 + _G * adv, P)

        lax.fori_loop(0, A // _G, group, jnp.int32(0))
        pltpu.make_async_copy(xbuf, o_hbm, out_sem).wait()

    pl.run_scoped(body,
                  pltpu.SemaphoreType.DMA((nbulk + 4,)),
                  pltpu.SemaphoreType.DMA((2,)),
                  pltpu.SemaphoreType.DMA(()))


@jax.jit
def pallas_standalone__channel_attn_cbam__vision_kernel(
    x: jax.Array,
    w1: jax.Array,
    w2: jax.Array,
):
    B, H, W, C = x.shape
    r = w1.shape[1]
    nw = W // _LANES
    ng = C // _TR
    A = H * ng * nw // _S
    assert B == 1 and W % _LANES == 0 and C % _TR == 0 and r <= _LANES // 2
    assert A * _S == H * ng * nw and A == _BULK[-1] + 1 and A % _G == 0
    assert (ng * nw) % (_BLK * nw) == 0 and _O % 2 == 1 and _L1 % 2 == 1

    xt = jnp.transpose(x, (0, 1, 3, 2))
    xf = xt.reshape(H * ng, _TR, nw, _LANES).transpose(0, 2, 1, 3)
    xf = xf.reshape(A, _S * _TR, _LANES)
    w1t = jnp.transpose(w1)

    tab_tiles = ng * nw + max(_O + _L1, _PER + 1 - _L1)
    out = pl.pallas_call(
        functools.partial(_kernel, nw=nw),
        out_shape=jax.ShapeDtypeStruct(xf.shape, x.dtype),
        in_specs=[pl.BlockSpec(memory_space=pl.ANY)] * 3,
        out_specs=pl.BlockSpec(memory_space=pl.ANY),
        scratch_shapes=[
            pltpu.VMEM(xf.shape, x.dtype),
            pltpu.VMEM((r, C), w1.dtype),
            pltpu.VMEM((r, C), w2.dtype),
            pltpu.VMEM((C, _LANES), jnp.float32),
            pltpu.VMEM((C, _LANES), jnp.float32),
            pltpu.VMEM((ng, _TR, _LANES), jnp.float32),
            pltpu.VMEM((ng, _TR, _LANES), jnp.float32),
            pltpu.VMEM((tab_tiles * _TR, _LANES), jnp.float32),
            pltpu.SMEM((1,), jnp.int32),
        ],
        compiler_params=pltpu.CompilerParams(
            vmem_limit_bytes=100 * 1024 * 1024),
    )(xf, w1t, w2)
    out = out.reshape(H * ng, nw, _TR, _LANES).transpose(0, 2, 1, 3)
    return jnp.transpose(out.reshape(B, H, C, W), (0, 1, 3, 2))
```

```python
import functools

import jax
import jax.numpy as jnp
from jax import lax
import jax.experimental.pallas as pl
import jax.experimental.pallas.tpu as pltpu

_LANES = 128
_TR = 8
_S = 256
_BLK = 8
_U = 2
_BULK = (0, 20, 64, 90, 101, 105, 106, 107)
_K = 4
_NL = 6
_SUB = 6
_G = 6
_PER = 32
_O = 5
_L1 = 13
_RAMP = (1, 1, 4)


def _kernel(x_hbm, w1t_hbm, w2_hbm, o_hbm,
            xbuf, w1buf, w2buf, w1d_ref, w2d_ref, sum_ref, max_ref, tab_ref,
            flag_ref, *, nw):
    A = xbuf.shape[0]
    ng = sum_ref.shape[0]
    P = ng * nw
    nb = P // _BLK
    bpa = _S // _BLK
    brows = _BLK * _TR
    vrows = _S * _TR
    hrows = P * _TR
    grows = nw * _TR
    H = A * _S // P
    half = _LANES // 2
    ne = ng - _NL
    nbulk = len(_BULK) - 1
    f32 = jnp.float32
    bf16 = jnp.bfloat16

    def pieces(r0, r1):
        out = []
        while r0 < r1:
            a, r = divmod(r0, vrows)
            n = min(r1 - r0, vrows - r)
            out.append((a, r, n))
            r0 += n
        return out

    def body(in_sems, w_sems, out_sem):
        tail0 = _BULK[-1] * vrows

        def bulk_copy(i):
            sl = pl.ds(_BULK[i], _BULK[i + 1] - _BULK[i])
            return pltpu.make_async_copy(x_hbm.at[sl], xbuf.at[sl],
                                         in_sems.at[i])

        def tail_copies(ranges, sem):
            cs = []
            for r0, r1 in ranges:
                for a, r, n in pieces(max(r0, tail0), r1):
                    sl = (a, pl.ds(r, n))
                    cs.append(pltpu.make_async_copy(x_hbm.at[sl], xbuf.at[sl],
                                                    sem))
            return cs

        early = [(h * hrows, h * hrows + ne * grows) for h in range(H - _K, H)]
        late = [(h * hrows + ne * grows, (h + 1) * hrows)
                for h in range(H - _K, H)]
        assert (H - _K) * hrows <= tail0 <= late[0][0]
        e1_cs = tail_copies(early[:-1], in_sems.at[nbulk])
        e2_cs = tail_copies(early[-1:], in_sems.at[nbulk + 1])
        l1_cs = tail_copies(late[:-1], in_sems.at[nbulk + 2])
        l2_cs = tail_copies(late[-1:], in_sems.at[nbulk + 3])

        w1_copy = pltpu.make_async_copy(w1t_hbm, w1buf, w_sems.at[0])
        w2_copy = pltpu.make_async_copy(w2_hbm, w2buf, w_sems.at[1])
        bulk_copy(0).start()
        bulk_copy(1).start()
        w1_copy.start()
        w2_copy.start()

        flag_ref[0] = 1

        def prep_weights():
            r = w1buf.shape[0]
            w1_copy.wait()
            w2_copy.wait()
            row = lax.broadcasted_iota(jnp.int32, (r, _LANES), 0)
            col = lax.broadcasted_iota(jnp.int32, (r, _LANES), 1)
            dup = jnp.where((col == row) | (col == row + half), 1.0, 0.0)
            dup = dup.astype(bf16)
            tn = (((0,), (0,)), ((), ()))
            w1d_ref[...] = lax.dot_general(w1buf[...], dup, tn,
                                           preferred_element_type=f32)
            w2d_ref[...] = lax.dot_general(w2buf[...], dup, tn,
                                           preferred_element_type=f32)

        def accumulate(v, s, m):
            v = v.reshape(s.shape[0], nw, _TR, _LANES)
            ps, pm = v[:, 0], v[:, 0]
            for k in range(1, nw):
                ps = ps + v[:, k]
                pm = jnp.maximum(pm, v[:, k])
            return s + ps, jnp.maximum(m, pm)

        def load_block(beta):
            a = lax.shift_right_logical(beta, bpa.bit_length() - 1)
            r = pl.multiple_of(lax.bitwise_and(beta, bpa - 1) * brows, brows)
            return xbuf[a, pl.ds(r, brows), :].astype(f32)

        def reduce_rows(h0, h1):
            for g in range(nb // nw):
                gs = pl.ds(g * _BLK, _BLK)

                def step(t, c):
                    for k in range(_U):
                        b0 = (h0 + t * _U + k) * nb + g * nw
                        v = jnp.concatenate(
                            [load_block(b0 + i) for i in range(nw)], axis=0)
                        c = accumulate(v, *c)
                    return c

                if h0 == 0:
                    acc = (_BLK, _TR, _LANES)
                    init = (jnp.zeros(acc, f32), jnp.full(acc, -jnp.inf, f32))
                else:
                    init = (sum_ref[gs], max_ref[gs])
                s, m = lax.fori_loop(0, (h1 - h0) // _U, step, init)
                sum_ref[gs] = s
                max_ref[gs] = m

        def fold_static(hs, g0, g1, s, m):
            for h in hs:
                v = jnp.concatenate(
                    [xbuf[a, pl.ds(r, n), :].astype(f32) for a, r, n in
                     pieces(h * hrows + g0 * grows, h * hrows + g1 * grows)],
                    axis=0)
                s, m = accumulate(v, s, m)
            return s, m

        done = 0
        for i in range(nbulk):
            bulk_copy(i).wait()
            if i == 0:
                for k in range(2, nbulk):
                    bulk_copy(k).start()
                for c in e1_cs + e2_cs + l1_cs + l2_cs:
                    c.start()
            if i == 1:
                prep_weights()
            h1 = min(_BULK[i + 1] * vrows // hrows, H - _K)
            h1 -= (h1 - done) % _U
            reduce_rows(done, h1)
            done = h1
        assert done == H - _K

        inv_n = 1.0 / (H * nw * _LANES)

        def hidden_part(g0, s, m):
            n = s.shape[0]
            s = s.reshape(n * _TR, _LANES)
            m = m.reshape(n * _TR, _LANES)
            gap = jnp.sum(s, axis=1, keepdims=True) * inv_n
            gmp = jnp.max(m, axis=1, keepdims=True)
            lane = lax.broadcasted_iota(jnp.int32, s.shape, 1)
            g = jnp.where(lane < half, gap, gmp).astype(bf16).astype(f32)
            hp = g * w1d_ref[pl.ds(g0 * _TR, n * _TR), :]
            parts = [hp[k * _TR:(k + 1) * _TR] for k in range(n)]
            while len(parts) > 1:
                parts = [parts[k] + parts[k + 1] if k + 1 < len(parts)
                         else parts[k] for k in range(0, len(parts), 2)]
            return parts[0]

        subs = [(g0, min(g0 + _SUB, ne)) for g0 in range(0, ne, _SUB)]
        for c in e1_cs:
            c.wait()
        for g0, g1 in subs:
            gs = pl.ds(g0, g1 - g0)
            s, m = fold_static(range(H - _K, H - 1), g0, g1,
                               sum_ref[gs], max_ref[gs])
            sum_ref[gs] = s
            max_ref[gs] = m
        for c in e2_cs:
            c.wait()
        hacc = None
        for g0, g1 in subs:
            gs = pl.ds(g0, g1 - g0)
            s, m = fold_static([H - 1], g0, g1, sum_ref[gs], max_ref[gs])
            p = hidden_part(g0, s, m)
            hacc = p if hacc is None else hacc + p
        for c in l1_cs:
            c.wait()
        gs = pl.ds(ne, _NL)
        s, m = fold_static(range(H - _K, H - 1), ne, ng,
                           sum_ref[gs], max_ref[gs])
        for c in l2_cs:
            c.wait()
        s, m = fold_static([H - 1], ne, ng, s, m)
        hacc = hacc + hidden_part(ne, s, m)
        h = jnp.sum(hacc, axis=0, keepdims=True)
        h = jnp.maximum(h.astype(bf16).astype(f32), 0.0)

        l2 = _PER - _L1
        es = _O + _L1
        order = (list(range(1, es // nw + 1)) + [0]
                 + list(range(es // nw + 1, ng)))
        sc_g = {}
        for k in order:
            z = jnp.sum(w2d_ref[pl.ds(k * _TR, _TR), :] * h, axis=1,
                        keepdims=True)
            z = jnp.broadcast_to(z, (_TR, _LANES)).astype(bf16).astype(f32)
            sg = (jnp.exp(jnp.minimum(z, 0.0))
                  * (0.5 * jnp.tanh(0.5 * jnp.abs(z)) + 0.5))
            sc_g[k] = sg.astype(bf16).astype(f32)

        def write(a0, na, b0, n):
            sl = (pl.ds(a0, na), pl.ds(b0 * _TR, n * _TR))
            pltpu.make_async_copy(xbuf.at[sl], o_hbm.at[sl], out_sem).start()

        def head_static(a0, n):
            rs = pl.ds(0, es * _TR)
            for a in range(a0, a0 + n):
                sc = jnp.concatenate(
                    [sc_g[((a * _S + t) // nw) % ng] for t in range(es)],
                    axis=0)
                xbuf[a, rs, :] = (xbuf[a, rs, :].astype(f32) * sc).astype(bf16)
            write(a0, n, _O, _L1)
            write(a0, n, 0, _O)

        head_static(0, _RAMP[0])

        @pl.when(flag_ref[0] == 1)
        def _():
            a0 = _RAMP[0]
            for n in _RAMP[1:]:
                head_static(a0, n)
                a0 += n
            assert a0 == _G

        @pl.when(flag_ref[0] == 1)
        def _():
            for t in range(tab_ref.shape[0] // _TR):
                tab_ref[pl.ds(t * _TR, _TR), :] = sc_g[(t // nw) % ng]

        adv = _S % P

        def scale_block(a0, pos0, e0, n):
            p = lax.rem(pos0 + e0, P)
            r0 = e0 * _TR
            if not isinstance(r0, int):
                r0 = pl.multiple_of(r0, 2 * _TR)
            rs = pl.ds(r0, n * _TR)
            for j in range(_G):
                sc = tab_ref[pl.ds(pl.multiple_of(p * _TR, _TR), n * _TR), :]
                xbuf[a0 + j, rs, :] = (
                    xbuf[a0 + j, rs, :].astype(f32) * sc).astype(bf16)
                p = p + adv
                p = jnp.where(p >= P, p - P, p)

        nper = (_S - es) // _PER
        last = es + _PER * nper

        def group(g, pos0):
            a0 = g * _G

            @pl.when(g > 0)
            def _():
                scale_block(a0, pos0, 0, es)
                write(a0, _G, 0, _O)
                write(a0, _G, _O, _L1)

            def period(mi, _):
                e0 = es + _PER * mi
                scale_block(a0, pos0, e0, l2 + 1)
                write(a0, _G, e0, l2)
                scale_block(a0, pos0, e0 + l2 + 1, _L1 - 1)
                write(a0, _G, e0 + l2, _L1)
                return 0

            lax.fori_loop(0, nper, period, 0)
            scale_block(a0, pos0, last, _S - last)
            write(a0, _G, last, _S - last)
            return lax.rem(pos0 + _G * adv, P)

        lax.fori_loop(0, A // _G, group, jnp.int32(0))
        pltpu.make_async_copy(xbuf, o_hbm, out_sem).wait()

    pl.run_scoped(body,
                  pltpu.SemaphoreType.DMA((nbulk + 4,)),
                  pltpu.SemaphoreType.DMA((2,)),
                  pltpu.SemaphoreType.DMA(()))


@jax.jit
def pallas_standalone__channel_attn_cbam__vision_kernel(
    x: jax.Array,
    w1: jax.Array,
    w2: jax.Array,
):
    B, H, W, C = x.shape
    r = w1.shape[1]
    nw = W // _LANES
    ng = C // _TR
    A = H * ng * nw // _S
    assert B == 1 and W % _LANES == 0 and C % _TR == 0 and r <= _LANES // 2
    assert A * _S == H * ng * nw and A == _BULK[-1] + 1 and A % _G == 0
    assert (ng * nw) % (_BLK * nw) == 0 and _O % 2 == 1 and _L1 % 2 == 1

    xt = jnp.transpose(x, (0, 1, 3, 2))
    xf = xt.reshape(H * ng, _TR, nw, _LANES).transpose(0, 2, 1, 3)
    xf = xf.reshape(A, _S * _TR, _LANES)
    w1t = jnp.transpose(w1)

    tab_tiles = ng * nw + max(_O + _L1, _PER + 1 - _L1)
    out = pl.pallas_call(
        functools.partial(_kernel, nw=nw),
        out_shape=jax.ShapeDtypeStruct(xf.shape, x.dtype),
        in_specs=[pl.BlockSpec(memory_space=pl.ANY)] * 3,
        out_specs=pl.BlockSpec(memory_space=pl.ANY),
        scratch_shapes=[
            pltpu.VMEM(xf.shape, x.dtype),
            pltpu.VMEM((r, C), w1.dtype),
            pltpu.VMEM((r, C), w2.dtype),
            pltpu.VMEM((C, _LANES), jnp.float32),
            pltpu.VMEM((C, _LANES), jnp.float32),
            pltpu.VMEM((ng, _TR, _LANES), jnp.float32),
            pltpu.VMEM((ng, _TR, _LANES), jnp.float32),
            pltpu.VMEM((tab_tiles * _TR, _LANES), jnp.float32),
            pltpu.SMEM((1,), jnp.int32),
        ],
        compiler_params=pltpu.CompilerParams(
            vmem_limit_bytes=100 * 1024 * 1024),
    )(xf, w1t, w2)
    out = out.reshape(H * ng, nw, _TR, _LANES).transpose(0, 2, 1, 3)
    return jnp.transpose(out.reshape(B, H, C, W), (0, 1, 3, 2))
```

```python
import functools

import jax
import jax.numpy as jnp
from jax import lax
import jax.experimental.pallas as pl
import jax.experimental.pallas.tpu as pltpu

_LANES = 128
_TR = 8
_S = 256
_BLK = 8
_U = 2
_BULK = (0, 20, 64, 90, 101, 105, 106, 107)
_K = 4
_NL = 6
_SUB = 6
_G = 6
_PER = 32
_O = 5
_L1 = 13
_RAMP = (1, 1, 4)


def _kernel(x_hbm, w1t_hbm, w2_hbm, o_hbm,
            xbuf, w1buf, w2buf, w1d_ref, w2d_ref, sum_ref, max_ref, tab_ref,
            sc_ref, *, nw):
    A = xbuf.shape[0]
    ng = sum_ref.shape[0]
    P = ng * nw
    nb = P // _BLK
    bpa = _S // _BLK
    brows = _BLK * _TR
    vrows = _S * _TR
    hrows = P * _TR
    grows = nw * _TR
    H = A * _S // P
    half = _LANES // 2
    ne = ng - _NL
    nbulk = len(_BULK) - 1
    f32 = jnp.float32
    bf16 = jnp.bfloat16

    def pieces(r0, r1):
        out = []
        while r0 < r1:
            a, r = divmod(r0, vrows)
            n = min(r1 - r0, vrows - r)
            out.append((a, r, n))
            r0 += n
        return out

    def body(in_sems, w_sems, out_sem):
        tail0 = _BULK[-1] * vrows

        def bulk_copy(i):
            sl = pl.ds(_BULK[i], _BULK[i + 1] - _BULK[i])
            return pltpu.make_async_copy(x_hbm.at[sl], xbuf.at[sl],
                                         in_sems.at[i])

        def tail_copies(ranges, sem):
            cs = []
            for r0, r1 in ranges:
                for a, r, n in pieces(max(r0, tail0), r1):
                    sl = (a, pl.ds(r, n))
                    cs.append(pltpu.make_async_copy(x_hbm.at[sl], xbuf.at[sl],
                                                    sem))
            return cs

        early = [(h * hrows, h * hrows + ne * grows) for h in range(H - _K, H)]
        late = [(h * hrows + ne * grows, (h + 1) * hrows)
                for h in range(H - _K, H)]
        assert (H - _K) * hrows <= tail0 <= late[0][0]
        e1_cs = tail_copies(early[:-1], in_sems.at[nbulk])
        e2_cs = tail_copies(early[-1:], in_sems.at[nbulk + 1])
        l1_cs = tail_copies(late[:-1], in_sems.at[nbulk + 2])
        l2_cs = tail_copies(late[-1:], in_sems.at[nbulk + 3])

        w1_copy = pltpu.make_async_copy(w1t_hbm, w1buf, w_sems.at[0])
        w2_copy = pltpu.make_async_copy(w2_hbm, w2buf, w_sems.at[1])
        bulk_copy(0).start()
        bulk_copy(1).start()
        w1_copy.start()
        w2_copy.start()

        def prep_weights():
            r = w1buf.shape[0]
            w1_copy.wait()
            w2_copy.wait()
            row = lax.broadcasted_iota(jnp.int32, (r, _LANES), 0)
            col = lax.broadcasted_iota(jnp.int32, (r, _LANES), 1)
            dup = jnp.where((col == row) | (col == row + half), 1.0, 0.0)
            dup = dup.astype(bf16)
            tn = (((0,), (0,)), ((), ()))
            w1d_ref[...] = lax.dot_general(w1buf[...], dup, tn,
                                           preferred_element_type=f32)
            w2d_ref[...] = lax.dot_general(w2buf[...], dup, tn,
                                           preferred_element_type=f32)

        def accumulate(v, s, m):
            v = v.reshape(s.shape[0], nw, _TR, _LANES)
            ps, pm = v[:, 0], v[:, 0]
            for k in range(1, nw):
                ps = ps + v[:, k]
                pm = jnp.maximum(pm, v[:, k])
            return s + ps, jnp.maximum(m, pm)

        def load_block(beta):
            a = lax.shift_right_logical(beta, bpa.bit_length() - 1)
            r = pl.multiple_of(lax.bitwise_and(beta, bpa - 1) * brows, brows)
            return xbuf[a, pl.ds(r, brows), :].astype(f32)

        def reduce_rows(h0, h1):
            for g in range(nb // nw):
                gs = pl.ds(g * _BLK, _BLK)

                def step(t, c):
                    for k in range(_U):
                        b0 = (h0 + t * _U + k) * nb + g * nw
                        v = jnp.concatenate(
                            [load_block(b0 + i) for i in range(nw)], axis=0)
                        c = accumulate(v, *c)
                    return c

                if h0 == 0:
                    acc = (_BLK, _TR, _LANES)
                    init = (jnp.zeros(acc, f32), jnp.full(acc, -jnp.inf, f32))
                else:
                    init = (sum_ref[gs], max_ref[gs])
                s, m = lax.fori_loop(0, (h1 - h0) // _U, step, init)
                sum_ref[gs] = s
                max_ref[gs] = m

        def fold_static(hs, g0, g1, s, m):
            for h in hs:
                v = jnp.concatenate(
                    [xbuf[a, pl.ds(r, n), :].astype(f32) for a, r, n in
                     pieces(h * hrows + g0 * grows, h * hrows + g1 * grows)],
                    axis=0)
                s, m = accumulate(v, s, m)
            return s, m

        done = 0
        for i in range(nbulk):
            bulk_copy(i).wait()
            if i == 0:
                for k in range(2, nbulk):
                    bulk_copy(k).start()
                for c in e1_cs + e2_cs + l1_cs + l2_cs:
                    c.start()
            if i == 1:
                prep_weights()
            h1 = min(_BULK[i + 1] * vrows // hrows, H - _K)
            h1 -= (h1 - done) % _U
            reduce_rows(done, h1)
            done = h1
        assert done == H - _K

        inv_n = 1.0 / (H * nw * _LANES)

        def hidden_part(g0, s, m):
            n = s.shape[0]
            s = s.reshape(n * _TR, _LANES)
            m = m.reshape(n * _TR, _LANES)
            gap = jnp.sum(s, axis=1, keepdims=True) * inv_n
            gmp = jnp.max(m, axis=1, keepdims=True)
            lane = lax.broadcasted_iota(jnp.int32, s.shape, 1)
            g = jnp.where(lane < half, gap, gmp).astype(bf16).astype(f32)
            hp = g * w1d_ref[pl.ds(g0 * _TR, n * _TR), :]
            parts = [hp[k * _TR:(k + 1) * _TR] for k in range(n)]
            while len(parts) > 1:
                parts = [parts[k] + parts[k + 1] if k + 1 < len(parts)
                         else parts[k] for k in range(0, len(parts), 2)]
            return parts[0]

        subs = [(g0, min(g0 + _SUB, ne)) for g0 in range(0, ne, _SUB)]
        for c in e1_cs:
            c.wait()
        for g0, g1 in subs:
            gs = pl.ds(g0, g1 - g0)
            s, m = fold_static(range(H - _K, H - 1), g0, g1,
                               sum_ref[gs], max_ref[gs])
            sum_ref[gs] = s
            max_ref[gs] = m
        for c in e2_cs:
            c.wait()
        hacc = None
        for g0, g1 in subs:
            gs = pl.ds(g0, g1 - g0)
            s, m = fold_static([H - 1], g0, g1, sum_ref[gs], max_ref[gs])
            p = hidden_part(g0, s, m)
            hacc = p if hacc is None else hacc + p
        for c in l1_cs:
            c.wait()
        gs = pl.ds(ne, _NL)
        s, m = fold_static(range(H - _K, H - 1), ne, ng,
                           sum_ref[gs], max_ref[gs])
        for c in l2_cs:
            c.wait()
        s, m = fold_static([H - 1], ne, ng, s, m)
        hacc = hacc + hidden_part(ne, s, m)
        h = jnp.sum(hacc, axis=0, keepdims=True)
        h = jnp.maximum(h.astype(bf16).astype(f32), 0.0)

        l2 = _PER - _L1
        es = _O + _L1
        order = (list(range(1, es // nw + 1)) + [0]
                 + list(range(es // nw + 1, ng)))
        sc_g = {}
        for k in order:
            z = jnp.sum(w2d_ref[pl.ds(k * _TR, _TR), :] * h, axis=1,
                        keepdims=True)
            z = jnp.broadcast_to(z, (_TR, _LANES)).astype(bf16).astype(f32)
            sg = (jnp.exp(jnp.minimum(z, 0.0))
                  * (0.5 * jnp.tanh(0.5 * jnp.abs(z)) + 0.5))
            sc_g[k] = sg.astype(bf16).astype(f32)

        def write(a0, na, b0, n):
            sl = (pl.ds(a0, na), pl.ds(b0 * _TR, n * _TR))
            pltpu.make_async_copy(xbuf.at[sl], o_hbm.at[sl], out_sem).start()

        def head_static(a0, n, sc_of):
            rs = pl.ds(0, es * _TR)
            for a in range(a0, a0 + n):
                sc = jnp.concatenate(
                    [sc_of[((a * _S + t) // nw) % ng] for t in range(es)],
                    axis=0)
                xbuf[a, rs, :] = (xbuf[a, rs, :].astype(f32) * sc).astype(bf16)
            write(a0, n, _O, _L1)
            write(a0, n, 0, _O)

        head_static(0, _RAMP[0], sc_g)
        for k in order:
            sc_ref[k] = sc_g[k]

        adv = _S % P

        def scale_block(a0, pos0, e0, n):
            p = lax.rem(pos0 + e0, P)
            r0 = e0 * _TR
            if not isinstance(r0, int):
                r0 = pl.multiple_of(r0, 2 * _TR)
            rs = pl.ds(r0, n * _TR)
            for j in range(_G):
                sc = tab_ref[pl.ds(pl.multiple_of(p * _TR, _TR), n * _TR), :]
                xbuf[a0 + j, rs, :] = (
                    xbuf[a0 + j, rs, :].astype(f32) * sc).astype(bf16)
                p = p + adv
                p = jnp.where(p >= P, p - P, p)

        nper = (_S - es) // _PER
        last = es + _PER * nper

        def group(g, pos0):
            a0 = g * _G

            @pl.when(g == 0)
            def _():
                sc_all = [sc_ref[k] for k in range(ng)]
                a = _RAMP[0]
                for n in _RAMP[1:]:
                    head_static(a, n, sc_all)
                    a += n
                assert a == _G

            @pl.when(g == 0)
            def _():
                for k in range(ng):
                    v = sc_ref[k]
                    for t in range(tab_ref.shape[0] // _TR):
                        if (t // nw) % ng == k:
                            tab_ref[pl.ds(t * _TR, _TR), :] = v

            @pl.when(g > 0)
            def _():
                scale_block(a0, pos0, 0, es)
                write(a0, _G, 0, _O)
                write(a0, _G, _O, _L1)

            def period(mi, _):
                e0 = es + _PER * mi
                scale_block(a0, pos0, e0, l2 + 1)
                write(a0, _G, e0, l2)
                scale_block(a0, pos0, e0 + l2 + 1, _L1 - 1)
                write(a0, _G, e0 + l2, _L1)
                return 0

            lax.fori_loop(0, nper, period, 0)
            scale_block(a0, pos0, last, _S - last)
            write(a0, _G, last, _S - last)
            return lax.rem(pos0 + _G * adv, P)

        lax.fori_loop(0, A // _G, group, jnp.int32(0))
        pltpu.make_async_copy(xbuf, o_hbm, out_sem).wait()

    pl.run_scoped(body,
                  pltpu.SemaphoreType.DMA((nbulk + 4,)),
                  pltpu.SemaphoreType.DMA((2,)),
                  pltpu.SemaphoreType.DMA(()))


@jax.jit
def pallas_standalone__channel_attn_cbam__vision_kernel(
    x: jax.Array,
    w1: jax.Array,
    w2: jax.Array,
):
    B, H, W, C = x.shape
    r = w1.shape[1]
    nw = W // _LANES
    ng = C // _TR
    A = H * ng * nw // _S
    assert B == 1 and W % _LANES == 0 and C % _TR == 0 and r <= _LANES // 2
    assert A * _S == H * ng * nw and A == _BULK[-1] + 1 and A % _G == 0
    assert (ng * nw) % (_BLK * nw) == 0 and _O % 2 == 1 and _L1 % 2 == 1

    xt = jnp.transpose(x, (0, 1, 3, 2))
    xf = xt.reshape(H * ng, _TR, nw, _LANES).transpose(0, 2, 1, 3)
    xf = xf.reshape(A, _S * _TR, _LANES)
    w1t = jnp.transpose(w1)

    tab_tiles = ng * nw + max(_O + _L1, _PER + 1 - _L1)
    out = pl.pallas_call(
        functools.partial(_kernel, nw=nw),
        out_shape=jax.ShapeDtypeStruct(xf.shape, x.dtype),
        in_specs=[pl.BlockSpec(memory_space=pl.ANY)] * 3,
        out_specs=pl.BlockSpec(memory_space=pl.ANY),
        scratch_shapes=[
            pltpu.VMEM(xf.shape, x.dtype),
            pltpu.VMEM((r, C), w1.dtype),
            pltpu.VMEM((r, C), w2.dtype),
            pltpu.VMEM((C, _LANES), jnp.float32),
            pltpu.VMEM((C, _LANES), jnp.float32),
            pltpu.VMEM((ng, _TR, _LANES), jnp.float32),
            pltpu.VMEM((ng, _TR, _LANES), jnp.float32),
            pltpu.VMEM((tab_tiles * _TR, _LANES), jnp.float32),
            pltpu.VMEM((ng, _TR, _LANES), jnp.float32),
        ],
        compiler_params=pltpu.CompilerParams(
            vmem_limit_bytes=100 * 1024 * 1024),
    )(xf, w1t, w2)
    out = out.reshape(H * ng, nw, _TR, _LANES).transpose(0, 2, 1, 3)
    return jnp.transpose(out.reshape(B, H, C, W), (0, 1, 3, 2))
```
